```python
import os as _os
_os.environ.setdefault("JAX_PLATFORMS", "cpu")
import jax
import jax.numpy as jnp

def _softmax(x, axis=-1):
    return jax.nn.softmax(x, axis=axis)
def _gelu(x):
    return jax.nn.gelu(x, approximate=True)
def _silu(x):
    return jax.nn.silu(x)
def _sigmoid(x):
    return jax.nn.sigmoid(x)
def _layernorm(x, axis=-1, eps=1e-5):
    m = jnp.mean(x, axis=axis, keepdims=True)
    v = jnp.var(x, axis=axis, keepdims=True)
    return (x - m) / jnp.sqrt(v + eps)
def _scatter_add(tgt, idx, src, axis=0):
    return tgt.at[idx].add(src)
def _segment_sum(src, seg, n):
    return jax.ops.segment_sum(src, seg, n)
class _Rng:
    def __init__(self, key):
        self._k = key
    def _next(self):
        self._k, sub = jax.random.split(self._k)
        return sub
    def normal(self, shape):
        return jax.random.normal(self._next(), shape, dtype=jnp.bfloat16)
    def randint(self, lo, hi, shape):
        return jax.random.randint(self._next(), shape, lo, hi, dtype=jnp.int32)
    def uniform(self, shape, lo=0.0, hi=1.0):
        return jax.random.uniform(self._next(), shape, jnp.bfloat16, lo, hi)
    def permutation(self, n):
        return jax.random.permutation(self._next(), n)


kernel_name = 'standalone__gqa_block_cached__near_ridge'

def setup_inputs():
    _rng = _Rng(jax.random.key(int.from_bytes(__import__("os").urandom(4), "little")))
    _w = (lambda a: (lambda t: t.astype(jnp.bfloat16) if jnp.issubdtype(t.dtype, jnp.floating) else t)(jnp.asarray(a)))
    B, Sq, D = 32, 112, 448
    Hq, Hkv, Sk, Dh = 16, 8, 512, 256
    assert Hq % Hkv == 0, (Hq, Hkv)
    return {
        "x": _w((lambda *s: _rng.normal(s) * 0.8)(B, Sq, D)),
        "k_cache": _w((lambda *s: _rng.normal(s) * 0.8)(B, Hkv, Sk, Dh)),
        "v_cache": _w((lambda *s: _rng.normal(s) * 0.05)(B, Hkv, Sk, Dh)),
        "wq": _w((lambda *s: _rng.normal(s) * 0.8)(D, Hq * Dh) * (D ** -0.5)),
        "wo": _w((lambda *s: _rng.normal(s) * 0.05)(Hq * Dh, D) * ((Hq * Dh) ** -0.5)),
    }

def reference(x, k_cache, v_cache, wq, wo):
    B, Sq, D = x.shape
    Hq, Dh = 16, 256
    Hkv = k_cache.shape[1]
    rep = Hq // Hkv
    q = (lambda x, *d: x.transpose(*d))((x @ wq).reshape(B, Sq, Hq, Dh), 0, 2, 1, 3)
    k = jnp.repeat(k_cache, rep, axis=1)
    v = jnp.repeat(v_cache, rep, axis=1)
    scores = jnp.einsum("bhqd,bhkd->bhqk", q, k) * (Dh ** -0.5)
    p = _softmax(scores, axis=-1)
    o = jnp.einsum("bhqk,bhkd->bhqd", p, v)
    return (lambda x, *d: x.transpose(*d))(o, 0, 2, 1, 3).reshape(B, Sq, Hq * Dh) @ wo
```

```python
import jax
import jax.numpy as jnp
import jax.experimental.pallas as pl
import jax.experimental.pallas.tpu as pltpu

HQ = 16
DH = 256
G = 2


def _kernel(x_ref, k_ref, v_ref, wq_ref, wo_ref, o_ref, q_sc, o_sc):
    g, sq, d = x_ref.shape
    hkv = k_ref.shape[1]
    rep = HQ // hkv
    scale = DH ** -0.5
    x = x_ref[...].reshape(g * sq, d)
    for h in range(HQ):
        qh = jnp.dot(x, wq_ref[:, h * DH:(h + 1) * DH], preferred_element_type=jnp.float32)
        qh = (qh * scale).astype(jnp.bfloat16)
        for b in range(g):
            q_sc[b, h // rep, (h % rep) * sq:(h % rep + 1) * sq, :] = qh[b * sq:(b + 1) * sq]
    for b in range(g):
        for h in range(hkv):
            q = q_sc[b, h]
            s = jax.lax.dot_general(q, k_ref[b, h], (((1,), (1,)), ((), ())),
                                    preferred_element_type=jnp.float32)
            m = jnp.max(s, axis=-1, keepdims=True)
            p = jnp.exp(s - m)
            l = jnp.sum(p, axis=-1, keepdims=True)
            o = jnp.dot(p.astype(jnp.bfloat16), v_ref[b, h], preferred_element_type=jnp.float32)
            o = (o / l).astype(jnp.bfloat16)
            for r in range(rep):
                hh = h * rep + r
                o_sc[b * sq:(b + 1) * sq, hh * DH:(hh + 1) * DH] = o[r * sq:(r + 1) * sq]
    out = jnp.dot(o_sc[...], wo_ref[...], preferred_element_type=jnp.float32)
    o_ref[...] = out.reshape(g, sq, d).astype(o_ref.dtype)


@jax.jit
def pallas_standalone__gqa_block_cached__near_ridge_kernel(x, k_cache, v_cache, wq, wo):
    B, Sq, D = x.shape
    _, Hkv, Sk, Dh = k_cache.shape
    rep = HQ // Hkv
    return pl.pallas_call(
        _kernel,
        grid=(B // G,),
        in_specs=[
            pl.BlockSpec((G, Sq, D), lambda i: (i, 0, 0)),
            pl.BlockSpec((G, Hkv, Sk, Dh), lambda i: (i, 0, 0, 0)),
            pl.BlockSpec((G, Hkv, Sk, Dh), lambda i: (i, 0, 0, 0)),
            pl.BlockSpec((D, HQ * Dh), lambda i: (0, 0)),
            pl.BlockSpec((HQ * Dh, D), lambda i: (0, 0)),
        ],
        out_specs=pl.BlockSpec((G, Sq, D), lambda i: (i, 0, 0)),
        out_shape=jax.ShapeDtypeStruct((B, Sq, D), x.dtype),
        scratch_shapes=[
            pltpu.VMEM((G, Hkv, rep * Sq, Dh), jnp.bfloat16),
            pltpu.VMEM((G * Sq, HQ * Dh), jnp.bfloat16),
        ],
        compiler_params=pltpu.CompilerParams(
            dimension_semantics=("arbitrary",),
            vmem_limit_bytes=100 * 1024 * 1024,
        ),
    )(x, k_cache, v_cache, wq, wo)
```

```python
import contextlib
import functools
import os
import jax
import jax.numpy as jnp
from jax import lax
import jax.experimental.pallas as pl
import jax.experimental.pallas.tpu as pltpu

HQ = 16
GS = 8
US = tuple(int(c) for c in os.environ.get('KU', '2222'))
MERGE = bool(int(os.environ.get('KMERGE', '0')))
SCOPES = bool(int(os.environ.get('KSC', '0')))
EPI = tuple(int(c) for c in os.environ.get('KEPI', '36').split(',')[0])
LOG2E = 1.4426950408889634
NT = (((1,), (1,)), ((), ()))
TT = 128


def scope(name):
    return jax.named_scope(name) if SCOPES else contextlib.nullcontext()


def _kernel(x_hbm, k_hbm, v_hbm, wq_hbm, wo_hbm, out_hbm,
            x_sc, wq_sc, wo_sc, q_sc0, q_sc1, o_sc0, o_sc1, acc0, acc1, out_sc, k_buf, v_buf,
            sem_x, sem_wq, sem_wo, sem_kv, sem_out, *, B, Sq):
    hkv, sk, dh = k_hbm.shape[1:]
    rep = HQ // hkv
    ng = B // GS
    gt = GS * Sq
    ntt = gt // TT
    cw = rep * dh
    d = x_hbm.shape[1]
    qscale = (dh ** -0.5) * LOG2E
    bf = jnp.bfloat16
    hx = gt // 2
    q_scs, o_scs, accs = (q_sc0, q_sc1), (o_sc0, o_sc1), (acc0, acc1)

    def x_copy(g):
        return pltpu.make_async_copy(x_hbm.at[pl.ds(g * gt, gt)], x_sc.at[g], sem_x.at[g])

    def x0_copy(half):
        return pltpu.make_async_copy(x_hbm.at[pl.ds(half * hx, hx)], x_sc.at[0, pl.ds(half * hx, hx)],
                                     sem_x.at[ng * half])

    def wq_copy(j):
        return pltpu.make_async_copy(wq_hbm.at[:, pl.ds(j * cw, cw)], wq_sc.at[j], sem_wq.at[j])

    def wo_copy(j):
        return pltpu.make_async_copy(wo_hbm.at[:, pl.ds(j * cw, cw)], wo_sc.at[j], sem_wo.at[j])

    def k_copy(g, j):
        return pltpu.make_async_copy(k_hbm.at[g * GS + j], k_buf.at[j], sem_kv.at[0, j])

    def v_copy(g, j):
        return pltpu.make_async_copy(v_hbm.at[g * GS + j], v_buf.at[j], sem_kv.at[1, j])

    def out_copy(g, tt):
        return pltpu.make_async_copy(out_sc.at[g, pl.ds(tt * TT, TT)], out_hbm.at[pl.ds(g * gt + tt * TT, TT)],
                                     sem_out.at[g, tt])

    def out_copy_group(g):
        return pltpu.make_async_copy(out_sc.at[g], out_hbm.at[pl.ds(g * gt, gt)], sem_out.at[g, 0])

    def q_half(g, j, b, r):
        qs = jnp.dot(x_sc[g, b * Sq:(b + 1) * Sq, :], wq_sc[j, :, r * dh:(r + 1) * dh],
                     preferred_element_type=jnp.float32)
        q_scs[g % 2][b, j, r * Sq:(r + 1) * Sq, :] = (qs * qscale).astype(bf)

    def q_rows(g, j, b0, b1):
        qs = jnp.dot(x_sc[g, b0 * Sq:b1 * Sq, :], wq_sc[j], preferred_element_type=jnp.float32)
        qs = (qs * qscale).astype(bf)
        for b in range(b0, b1):
            for r in range(rep):
                q_scs[g % 2][b, j, r * Sq:(r + 1) * Sq, :] = qs[(b - b0) * Sq:(b - b0 + 1) * Sq, r * dh:(r + 1) * dh]

    def qk(g, j, h):
        return lax.dot_general(q_scs[g % 2][j, h], k_buf[j, h], NT, preferred_element_type=jnp.float32)

    def pv(g, j, h, s):
        row0 = pl.multiple_of(j * Sq, 16)
        m = jnp.max(s, axis=-1, keepdims=True)
        p = jnp.exp2(s - m)
        l = jnp.sum(p, axis=-1, keepdims=True)
        o = jnp.dot(p.astype(bf), v_buf[j, h], preferred_element_type=jnp.float32)
        r0 = pl.reciprocal(l, approx=True)
        r0 = r0 * (2.0 - l * r0)
        o = (o * r0).astype(bf)
        for r in range(rep):
            o_scs[g % 2][h, pl.ds(row0, Sq), r * dh:(r + 1) * dh] = o[r * Sq:(r + 1) * Sq]

    def o_piece(g, j, tt):
        part = lax.dot_general(wo_sc[j], o_scs[g % 2][j, tt * TT:(tt + 1) * TT, :], NT,
                               preferred_element_type=jnp.float32)
        accs[g % 2][tt] = jnp.where(j == 0, 0.0, accs[g % 2][tt]) + part

    def t_piece(g, tt):
        row0 = tt * TT if isinstance(tt, int) else pl.multiple_of(tt * TT, TT)
        out_sc[g, pl.ds(row0, TT), :] = accs[g % 2][tt].T.astype(bf)

    def start_loop(fn, lo, hi):
        def body(i, c):
            fn(i)
            return c
        lax.fori_loop(lo, hi, body, 0)

    def kv_start(g, j):
        k_copy(g, j).start()
        v_copy(g, j).start()

    wq_copy(0).start()
    start_loop(lambda h: x0_copy(h).start(), 0, 2)
    start_loop(lambda j: wq_copy(j).start(), 1, hkv)
    start_loop(lambda j: kv_start(0, j), 0, 2)
    x_copy(1).start()
    start_loop(lambda j: kv_start(0, j), 2, GS)
    start_loop(lambda j: wo_copy(j).start(), 0, hkv)
    start_loop(lambda g: x_copy(g).start(), 2, ng)
    with scope('pro0'):
        wq_copy(0).wait()
        x0_copy(0).wait()
        q_rows(0, 0, 0, GS // 2)
    PU = int(os.environ.get('KPU', '2'))
    first = 1 + (hkv - 1) % PU
    with scope('pro1'):
        x0_copy(1).wait()
        for j in range(1, first):
            wq_copy(j).wait()
        q_rows(0, 0, GS // 2, GS)
        for j in range(1, first):
            q_rows(0, j, 0, GS)

    def pbody(i, c):
        for a in range(PU):
            wq_copy(first + i * PU + a).wait()
        for a in range(PU):
            q_rows(0, first + i * PU + a, 0, GS)
        return c
    with scope('pro2'):
        lax.fori_loop(0, (hkv - first) // PU, pbody, 0)
    x_copy(1).wait()

    def step(g, i, U, do_q, do_o, do_t):
        with scope('kv_wait'):
            for u in range(U):
                k_copy(g, i * U + u).wait()
                v_copy(g, i * U + u).wait()

        with scope('compute'):
            for u in range(U):
                j = i * U + u
                qf = [functools.partial(q_half, g + 1, j, b, r) for b in range(GS) for r in range(rep)] if do_q else []
                of = [functools.partial(o_piece, g - 1, j, tt) for tt in range(ntt)] if do_o else []
                pre = [[] for _ in range(hkv)]
                mid = [[] for _ in range(hkv)]
                if do_q and do_o:
                    for h in range(hkv):
                        pre[h] = qf[2 * h:2 * h + 1]
                        mid[h] = qf[2 * h + 1:2 * h + 2] + of[h:h + 1]
                elif do_q:
                    for h in range(hkv):
                        pre[h] = qf[2 * h:2 * h + 1]
                        mid[h] = qf[2 * h + 1:2 * h + 2]
                elif do_o:
                    for h in range(hkv):
                        mid[h] = of[h - 1:h] if h > 0 else []
                if do_q or not do_o:
                    for h in range(hkv):
                        for f in pre[h]: f()
                        s = qk(g, j, h)
                        for f in mid[h]: f()
                        pv(g, j, h, s)
                else:
                    s0 = qk(g, j, 0)
                    s1 = qk(g, j, 1)
                    pv(g, j, 0, s0)
                    of[0]()
                    pv(g, j, 1, s1)
                    for h in range(2, hkv):
                        s = qk(g, j, h)
                        of[h - 1]()
                        pv(g, j, h, s)
                if do_t:
                    t_piece(g - 2, jnp.minimum(j, ntt - 1))

        if do_q:
            for u in range(U):
                kv_start(g + 1, i * U + u)

    def group_loop(g, U, do_q, do_o, do_t):
        def body(i, c):
            step(g, i, U, do_q, do_o, do_t)
            return c
        lax.fori_loop(0, GS // U, body, 0)

    for g in range(ng):
        if g == 1:
            for j in range(hkv):
                wo_copy(j).wait()
        if 1 <= g < ng - 1:
            x_copy(g + 1).wait()
        group_loop(g, US[g], g + 1 < ng, g >= 1, g >= 2)
        if g >= 2:
            out_copy_group(g - 2).start()

    g = ng - 1

    def o_tile(tt):
        row0 = tt * TT if isinstance(tt, int) else pl.multiple_of(tt * TT, TT)
        part = None
        for j in range(hkv):
            pj = lax.dot_general(wo_sc[j], o_scs[g % 2][j, pl.ds(row0, TT), :], NT,
                                 preferred_element_type=jnp.float32)
            part = pj if part is None else part + pj
        accs[g % 2][tt] = part

    EU = int(os.environ.get('KEU', '2'))
    efirst = 1 + (ntt - 1) % EU
    with scope('epi0'):
        for tt in range(ntt):
            t_piece(g - 1, tt)
        for tt in range(efirst):
            o_tile(tt)
        out_copy_group(g - 1).start()

    def ebody(i, c):
        t0 = efirst + i * EU
        prev = [t0 - EU + a for a in range(EU)]
        prev = [jnp.maximum(t, 0) for t in prev]
        for t in prev:
            t_piece(g, t)
        for a in range(EU):
            o_tile(t0 + a)
        return c
    with scope('epi1'):
        lax.fori_loop(0, (ntt - efirst) // EU, ebody, 0)
    with scope('epi2'):
        nprev = ntt - EU
        pltpu.make_async_copy(out_sc.at[g, pl.ds(0, nprev * TT)], out_hbm.at[pl.ds(g * gt, nprev * TT)],
                              sem_out.at[g, 0]).start()
        for tt in range(nprev, ntt):
            t_piece(g, tt)
            out_copy(g, tt).start()
    with scope('epi_out'):
        for gg in range(ng - 1):
            out_copy_group(gg).wait()
        pltpu.make_async_copy(out_sc.at[g, pl.ds(0, nprev * TT)], out_hbm.at[pl.ds(g * gt, nprev * TT)],
                              sem_out.at[g, 0]).wait()
        for tt in range(nprev, ntt):
            out_copy(g, tt).wait()


@jax.jit
def pallas_standalone__gqa_block_cached__near_ridge_kernel(x, k_cache, v_cache, wq, wo):
    B, Sq, D = x.shape
    _, Hkv, Sk, Dh = k_cache.shape
    rep = HQ // Hkv
    ng = B // GS
    gt = GS * Sq
    cw = rep * Dh
    bf = jnp.bfloat16
    any_spec = pl.BlockSpec(memory_space=pl.ANY)
    out = pl.pallas_call(
        functools.partial(_kernel, B=B, Sq=Sq),
        in_specs=[any_spec] * 5,
        out_specs=any_spec,
        out_shape=jax.ShapeDtypeStruct((B * Sq, D), x.dtype),
        scratch_shapes=[
            pltpu.VMEM((ng, gt, D), bf),
            pltpu.VMEM((Hkv, D, cw), bf),
            pltpu.VMEM((Hkv, D, cw), bf),
            pltpu.VMEM((GS, Hkv, rep * Sq, Dh), bf),
            pltpu.VMEM((GS, Hkv, rep * Sq, Dh), bf),
            pltpu.VMEM((Hkv, gt, cw), bf),
            pltpu.VMEM((Hkv, gt, cw), bf),
            pltpu.VMEM((gt // TT, D, TT), jnp.float32),
            pltpu.VMEM((gt // TT, D, TT), jnp.float32),
            pltpu.VMEM((ng, gt, D), bf),
            pltpu.VMEM((GS, Hkv, Sk, Dh), bf),
            pltpu.VMEM((GS, Hkv, Sk, Dh), bf),
            pltpu.SemaphoreType.DMA((ng + 1,)),
            pltpu.SemaphoreType.DMA((Hkv,)),
            pltpu.SemaphoreType.DMA((Hkv,)),
            pltpu.SemaphoreType.DMA((2, GS)),
            pltpu.SemaphoreType.DMA((ng, gt // TT)),
        ],
        compiler_params=pltpu.CompilerParams(vmem_limit_bytes=120 * 1024 * 1024,
                                             disable_bounds_checks=True),
    )(x.reshape(B * Sq, D), k_cache, v_cache, wq, wo.T)
    return out.reshape(B, Sq, D)
```

```python
import functools

import jax
import jax.numpy as jnp
from jax import lax
import jax.experimental.pallas as pl
import jax.experimental.pallas.tpu as pltpu

HQ = 16
GS = 8
U = 2
PU = 3
TT = 128
EPI = (6,)
LOG2E = 1.4426950408889634
NT = (((1,), (1,)), ((), ()))


def _kernel(x_hbm, k_hbm, v_hbm, wq_hbm, wo_hbm, out_hbm,
            x_sc, wq_sc, wo_sc, q_sc0, q_sc1, o_sc0, o_sc1, acc0, acc1, out_sc, k_buf, v_buf,
            sem_x, sem_wq, sem_wo, sem_kv, sem_out, *, B, Sq):
    hkv, _, dh = k_hbm.shape[1:]
    rep = HQ // hkv
    ng = B // GS
    gt = GS * Sq
    ntt = gt // TT
    cw = rep * dh
    hx = gt // 2
    qscale = (dh ** -0.5) * LOG2E
    bf = jnp.bfloat16
    q_scs, o_scs, accs = (q_sc0, q_sc1), (o_sc0, o_sc1), (acc0, acc1)

    def x_copy(g):
        return pltpu.make_async_copy(x_hbm.at[pl.ds(g * gt, gt)], x_sc.at[g], sem_x.at[g])

    def x0_copy(half):
        return pltpu.make_async_copy(x_hbm.at[pl.ds(half * hx, hx)], x_sc.at[0, pl.ds(half * hx, hx)],
                                     sem_x.at[ng * half])

    def wq_copy(j):
        return pltpu.make_async_copy(wq_hbm.at[:, pl.ds(j * cw, cw)], wq_sc.at[j], sem_wq.at[j])

    def wq0_copy(r):
        return pltpu.make_async_copy(wq_hbm.at[:, pl.ds(r * dh, dh)], wq_sc.at[0, :, pl.ds(r * dh, dh)],
                                     sem_wq.at[hkv * r])

    def wo_copy(j):
        return pltpu.make_async_copy(wo_hbm.at[:, pl.ds(j * cw, cw)], wo_sc.at[j], sem_wo.at[j])

    def k_copy(g, j):
        return pltpu.make_async_copy(k_hbm.at[g * GS + j], k_buf.at[j], sem_kv.at[0, j])

    def v_copy(g, j):
        return pltpu.make_async_copy(v_hbm.at[g * GS + j], v_buf.at[j], sem_kv.at[1, j])

    def out_copy(g, tt):
        return pltpu.make_async_copy(out_sc.at[g, pl.ds(tt * TT, TT)], out_hbm.at[pl.ds(g * gt + tt * TT, TT)],
                                     sem_out.at[g, tt])

    def out_copy_group(g):
        return pltpu.make_async_copy(out_sc.at[g], out_hbm.at[pl.ds(g * gt, gt)], sem_out.at[g, 0])

    def start_loop(fn, lo, hi):
        def body(i, c):
            fn(i)
            return c
        lax.fori_loop(lo, hi, body, 0)

    def kv_start(g, j):
        k_copy(g, j).start()
        v_copy(g, j).start()

    def q_part(g, j, b0, b1, r0, r1):
        qs = jnp.dot(x_sc[g, b0 * Sq:b1 * Sq, :], wq_sc[j, :, r0 * dh:r1 * dh],
                     preferred_element_type=jnp.float32)
        qs = (qs * qscale).astype(bf)
        for b in range(b0, b1):
            for r in range(r0, r1):
                q_scs[g % 2][b, j, r * Sq:(r + 1) * Sq, :] = (
                    qs[(b - b0) * Sq:(b - b0 + 1) * Sq, (r - r0) * dh:(r - r0 + 1) * dh])

    def qk(g, j, h):
        return lax.dot_general(q_scs[g % 2][j, h], k_buf[j, h], NT, preferred_element_type=jnp.float32)

    def pv(g, j, h, s):
        row0 = pl.multiple_of(j * Sq, 16)
        m = jnp.max(s, axis=-1, keepdims=True)
        p = jnp.exp2(s - m)
        l = jnp.sum(p, axis=-1, keepdims=True)
        o = jnp.dot(p.astype(bf), v_buf[j, h], preferred_element_type=jnp.float32)
        inv = pl.reciprocal(l, approx=True)
        inv = inv * (2.0 - l * inv)
        o = (o * inv).astype(bf)
        for r in range(rep):
            o_scs[g % 2][h, pl.ds(row0, Sq), r * dh:(r + 1) * dh] = o[r * Sq:(r + 1) * Sq]

    def o_piece(g, j, tt):
        part = lax.dot_general(wo_sc[j], o_scs[g % 2][j, tt * TT:(tt + 1) * TT, :], NT,
                               preferred_element_type=jnp.float32)
        accs[g % 2][tt] = jnp.where(j == 0, 0.0, accs[g % 2][tt]) + part

    def t_piece(g, tt):
        row0 = tt * TT if isinstance(tt, int) else pl.multiple_of(tt * TT, TT)
        out_sc[g, pl.ds(row0, TT), :] = accs[g % 2][tt].T.astype(bf)

    def first_start(h):
        wq0_copy(h).start()
        x0_copy(h).start()
    start_loop(first_start, 0, 2)
    start_loop(lambda j: wq_copy(j).start(), 1, hkv)
    start_loop(lambda j: kv_start(0, j), 0, U)
    x_copy(1).start()
    start_loop(lambda j: kv_start(0, j), U, GS)
    start_loop(lambda j: wo_copy(j).start(), 0, hkv)
    start_loop(lambda g: x_copy(g).start(), 2, ng)

    wq0_copy(0).wait()
    x0_copy(0).wait()
    q_part(0, 0, 0, GS // 2, 0, 1)
    wq0_copy(1).wait()
    q_part(0, 0, 0, GS // 2, 1, rep)
    x0_copy(1).wait()
    q_part(0, 0, GS // 2, GS, 0, rep)
    first = 1 + (hkv - 1) % PU
    for j in range(1, first):
        wq_copy(j).wait()
    for j in range(1, first):
        q_part(0, j, 0, GS, 0, rep)

    def pbody(i, c):
        for a in range(PU):
            wq_copy(first + i * PU + a).wait()
        for a in range(PU):
            q_part(0, first + i * PU + a, 0, GS, 0, rep)
        return c
    lax.fori_loop(0, (hkv - first) // PU, pbody, 0)
    x_copy(1).wait()

    def step(g, i):
        do_q, do_o, do_t = g + 1 < ng, g >= 1, g >= 2
        for u in range(U):
            k_copy(g, i * U + u).wait()
            v_copy(g, i * U + u).wait()

        for u in range(U):
            j = i * U + u
            qf = [functools.partial(q_part, g + 1, j, b, b + 1, r, r + 1)
                  for b in range(GS) for r in range(rep)] if do_q else []
            of = [functools.partial(o_piece, g - 1, j, tt) for tt in range(ntt)] if do_o else []
            if do_q:
                for h in range(hkv):
                    qf[2 * h]()
                    s = qk(g, j, h)
                    qf[2 * h + 1]()
                    if h < len(of):
                        of[h]()
                    pv(g, j, h, s)
            else:
                s0 = qk(g, j, 0)
                s1 = qk(g, j, 1)
                pv(g, j, 0, s0)
                of[0]()
                pv(g, j, 1, s1)
                for h in range(2, hkv):
                    s = qk(g, j, h)
                    of[h - 1]()
                    pv(g, j, h, s)
            if do_t:
                t_piece(g - 2, jnp.minimum(j, ntt - 1))

        if do_q:
            for u in range(U):
                kv_start(g + 1, i * U + u)

    for g in range(ng):
        if g == 1:
            for j in range(hkv):
                wo_copy(j).wait()
        if 1 <= g < ng - 1:
            x_copy(g + 1).wait()

        def body(i, c, g=g):
            step(g, i)
            return c
        lax.fori_loop(0, GS // U, body, 0)
        if g >= 2:
            out_copy_group(g - 2).start()

    g = ng - 1

    def o_tile(tt):
        part = None
        for j in range(hkv):
            pj = lax.dot_general(wo_sc[j], o_scs[g % 2][j, tt * TT:(tt + 1) * TT, :], NT,
                                 preferred_element_type=jnp.float32)
            part = pj if part is None else part + pj
        out_sc[g, tt * TT:(tt + 1) * TT, :] = part.T.astype(bf)

    bounds = (0,) + EPI + (ntt,)
    for si in range(len(bounds) - 1):
        if si == 0:
            for tt in range(ntt):
                t_piece(g - 1, tt)
        for tt in range(bounds[si], bounds[si + 1]):
            o_tile(tt)
        if si == 0:
            out_copy_group(g - 1).start()
        for tt in range(bounds[si], bounds[si + 1]):
            out_copy(g, tt).start()
        if si < len(bounds) - 2:
            out_copy_group(si).wait()
    for gg in range(len(bounds) - 2, ng - 1):
        out_copy_group(gg).wait()
    for tt in range(ntt):
        out_copy(g, tt).wait()


@jax.jit
def pallas_standalone__gqa_block_cached__near_ridge_kernel(x, k_cache, v_cache, wq, wo):
    B, Sq, D = x.shape
    _, Hkv, Sk, Dh = k_cache.shape
    rep = HQ // Hkv
    ng = B // GS
    gt = GS * Sq
    cw = rep * Dh
    bf = jnp.bfloat16
    any_spec = pl.BlockSpec(memory_space=pl.ANY)
    out = pl.pallas_call(
        functools.partial(_kernel, B=B, Sq=Sq),
        in_specs=[any_spec] * 5,
        out_specs=any_spec,
        out_shape=jax.ShapeDtypeStruct((B * Sq, D), x.dtype),
        scratch_shapes=[
            pltpu.VMEM((ng, gt, D), bf),
            pltpu.VMEM((Hkv, D, cw), bf),
            pltpu.VMEM((Hkv, D, cw), bf),
            pltpu.VMEM((GS, Hkv, rep * Sq, Dh), bf),
            pltpu.VMEM((GS, Hkv, rep * Sq, Dh), bf),
            pltpu.VMEM((Hkv, gt, cw), bf),
            pltpu.VMEM((Hkv, gt, cw), bf),
            pltpu.VMEM((gt // TT, D, TT), jnp.float32),
            pltpu.VMEM((gt // TT, D, TT), jnp.float32),
            pltpu.VMEM((ng, gt, D), bf),
            pltpu.VMEM((GS, Hkv, Sk, Dh), bf),
            pltpu.VMEM((GS, Hkv, Sk, Dh), bf),
            pltpu.SemaphoreType.DMA((ng + 1,)),
            pltpu.SemaphoreType.DMA((Hkv + 1,)),
            pltpu.SemaphoreType.DMA((Hkv,)),
            pltpu.SemaphoreType.DMA((2, GS)),
            pltpu.SemaphoreType.DMA((ng, gt // TT)),
        ],
        compiler_params=pltpu.CompilerParams(vmem_limit_bytes=120 * 1024 * 1024,
                                             disable_bounds_checks=True),
    )(x.reshape(B * Sq, D), k_cache, v_cache, wq, wo.T)
    return out.reshape(B, Sq, D)
```

```python
import functools

import jax
import jax.numpy as jnp
from jax import lax
import jax.experimental.pallas as pl
import jax.experimental.pallas.tpu as pltpu

HQ = 16
GS = 8
U = 2
PU = 3
TT = 128
EPI = (6,)
LOG2E = 1.4426950408889634
NT = (((1,), (1,)), ((), ()))


def _kernel(x_hbm, k_hbm, v_hbm, wq_hbm, wo_hbm, out_hbm,
            x_sc, wq_sc, wo_sc, q_sc0, q_sc1, o_sc0, o_sc1, acc0, acc1, out_sc, k_buf, v_buf,
            sem_x, sem_wq, sem_wo, sem_kv, sem_out, *, B, Sq):
    hkv, _, dh = k_hbm.shape[1:]
    rep = HQ // hkv
    ng = B // GS
    gt = GS * Sq
    ntt = gt // TT
    cw = rep * dh
    hx = gt // 2
    qscale = (dh ** -0.5) * LOG2E
    bf = jnp.bfloat16
    q_scs, o_scs, accs = (q_sc0, q_sc1), (o_sc0, o_sc1), (acc0, acc1)

    def x_copy(g):
        return pltpu.make_async_copy(x_hbm.at[pl.ds(g * gt, gt)], x_sc.at[g], sem_x.at[g])

    def x0_copy(half):
        return pltpu.make_async_copy(x_hbm.at[pl.ds(half * hx, hx)], x_sc.at[0, pl.ds(half * hx, hx)],
                                     sem_x.at[ng * half])

    def wq_copy(j):
        return pltpu.make_async_copy(wq_hbm.at[:, pl.ds(j * cw, cw)], wq_sc.at[j], sem_wq.at[j])

    def wq0_copy(r):
        return pltpu.make_async_copy(wq_hbm.at[:, pl.ds(r * dh, dh)], wq_sc.at[0, :, pl.ds(r * dh, dh)],
                                     sem_wq.at[hkv * r])

    def wo_copy(j):
        return pltpu.make_async_copy(wo_hbm.at[:, pl.ds(j * cw, cw)], wo_sc.at[j], sem_wo.at[j])

    def k_copy(g, i):
        return pltpu.make_async_copy(k_hbm.at[pl.ds(g * GS + i * U, U)], k_buf.at[pl.ds(i * U, U)], sem_kv.at[0, i])

    def v_copy(g, i):
        return pltpu.make_async_copy(v_hbm.at[pl.ds(g * GS + i * U, U)], v_buf.at[pl.ds(i * U, U)], sem_kv.at[1, i])

    def out_copy(g, tt):
        return pltpu.make_async_copy(out_sc.at[g, pl.ds(tt * TT, TT)], out_hbm.at[pl.ds(g * gt + tt * TT, TT)],
                                     sem_out.at[g, tt])

    def out_copy_group(g):
        return pltpu.make_async_copy(out_sc.at[g], out_hbm.at[pl.ds(g * gt, gt)], sem_out.at[g, 0])

    def start_loop(fn, lo, hi):
        def body(i, c):
            fn(i)
            return c
        lax.fori_loop(lo, hi, body, 0)

    def kv_start(g, i):
        k_copy(g, i).start()
        v_copy(g, i).start()

    def q_part(g, j, b0, b1, r0, r1):
        qs = jnp.dot(x_sc[g, b0 * Sq:b1 * Sq, :], wq_sc[j, :, r0 * dh:r1 * dh],
                     preferred_element_type=jnp.float32)
        qs = (qs * qscale).astype(bf)
        for b in range(b0, b1):
            for r in range(r0, r1):
                q_scs[g % 2][b, j, r * Sq:(r + 1) * Sq, :] = (
                    qs[(b - b0) * Sq:(b - b0 + 1) * Sq, (r - r0) * dh:(r - r0 + 1) * dh])

    def qk(g, j, h):
        return lax.dot_general(q_scs[g % 2][j, h], k_buf[j, h], NT, preferred_element_type=jnp.float32)

    def pv(g, j, h, s):
        row0 = pl.multiple_of(j * Sq, 16)
        m = jnp.max(s, axis=-1, keepdims=True)
        p = jnp.exp2(s - m)
        l = jnp.sum(p, axis=-1, keepdims=True)
        o = jnp.dot(p.astype(bf), v_buf[j, h], preferred_element_type=jnp.float32)
        inv = pl.reciprocal(l, approx=True)
        inv = inv * (2.0 - l * inv)
        o = (o * inv).astype(bf)
        for r in range(rep):
            o_scs[g % 2][h, pl.ds(row0, Sq), r * dh:(r + 1) * dh] = o[r * Sq:(r + 1) * Sq]

    def o_piece(g, j, tt):
        part = lax.dot_general(wo_sc[j], o_scs[g % 2][j, tt * TT:(tt + 1) * TT, :], NT,
                               preferred_element_type=jnp.float32)
        accs[g % 2][tt] = jnp.where(j == 0, 0.0, accs[g % 2][tt]) + part

    def t_piece(g, tt):
        row0 = tt * TT if isinstance(tt, int) else pl.multiple_of(tt * TT, TT)
        out_sc[g, pl.ds(row0, TT), :] = accs[g % 2][tt].T.astype(bf)

    def first_start(h):
        wq0_copy(h).start()
        x0_copy(h).start()
    start_loop(first_start, 0, 2)
    start_loop(lambda j: wq_copy(j).start(), 1, hkv)
    kv_start(0, 0)
    x_copy(1).start()
    start_loop(lambda i: kv_start(0, i), 1, GS // U)
    start_loop(lambda j: wo_copy(j).start(), 0, hkv)
    start_loop(lambda g: x_copy(g).start(), 2, ng)

    wq0_copy(0).wait()
    x0_copy(0).wait()
    q_part(0, 0, 0, GS // 2, 0, 1)
    wq0_copy(1).wait()
    q_part(0, 0, 0, GS // 2, 1, rep)
    x0_copy(1).wait()
    q_part(0, 0, GS // 2, GS, 0, rep)
    first = 1 + (hkv - 1) % PU
    for j in range(1, first):
        wq_copy(j).wait()
    for j in range(1, first):
        q_part(0, j, 0, GS, 0, rep)

    def pbody(i, c):
        for a in range(PU):
            wq_copy(first + i * PU + a).wait()
        for a in range(PU):
            q_part(0, first + i * PU + a, 0, GS, 0, rep)
        return c
    lax.fori_loop(0, (hkv - first) // PU, pbody, 0)
    x_copy(1).wait()

    def step(g, i):
        do_q, do_o, do_t = g + 1 < ng, g >= 1, g >= 2
        k_copy(g, i).wait()
        v_copy(g, i).wait()

        for u in range(U):
            j = i * U + u
            qf = [functools.partial(q_part, g + 1, j, b, b + 1, r, r + 1)
                  for b in range(GS) for r in range(rep)] if do_q else []
            of = [functools.partial(o_piece, g - 1, j, tt) for tt in range(ntt)] if do_o else []
            if do_q:
                for h in range(hkv):
                    qf[2 * h]()
                    s = qk(g, j, h)
                    qf[2 * h + 1]()
                    if h < len(of):
                        of[h]()
                    pv(g, j, h, s)
            else:
                s0 = qk(g, j, 0)
                s1 = qk(g, j, 1)
                pv(g, j, 0, s0)
                of[0]()
                pv(g, j, 1, s1)
                for h in range(2, hkv):
                    s = qk(g, j, h)
                    of[h - 1]()
                    pv(g, j, h, s)
            if do_t:
                t_piece(g - 2, jnp.minimum(j, ntt - 1))

        if do_q:
            kv_start(g + 1, i)

    for g in range(ng):
        if g == 1:
            for j in range(hkv):
                wo_copy(j).wait()
        if 1 <= g < ng - 1:
            x_copy(g + 1).wait()

        def body(i, c, g=g):
            step(g, i)
            return c
        lax.fori_loop(0, GS // U, body, 0)
        if g >= 2:
            out_copy_group(g - 2).start()

    g = ng - 1

    def o_tile(tt):
        part = None
        for j in range(hkv):
            pj = lax.dot_general(wo_sc[j], o_scs[g % 2][j, tt * TT:(tt + 1) * TT, :], NT,
                                 preferred_element_type=jnp.float32)
            part = pj if part is None else part + pj
        out_sc[g, tt * TT:(tt + 1) * TT, :] = part.T.astype(bf)

    bounds = (0,) + EPI + (ntt,)
    for si in range(len(bounds) - 1):
        if si == 0:
            for tt in range(ntt):
                t_piece(g - 1, tt)
        for tt in range(bounds[si], bounds[si + 1]):
            o_tile(tt)
        if si == 0:
            out_copy_group(g - 1).start()
        for tt in range(bounds[si], bounds[si + 1]):
            out_copy(g, tt).start()
        if si < len(bounds) - 2:
            out_copy_group(si).wait()
    for gg in range(len(bounds) - 2, ng - 1):
        out_copy_group(gg).wait()
    for tt in range(ntt):
        out_copy(g, tt).wait()


@jax.jit
def pallas_standalone__gqa_block_cached__near_ridge_kernel(x, k_cache, v_cache, wq, wo):
    B, Sq, D = x.shape
    _, Hkv, Sk, Dh = k_cache.shape
    rep = HQ // Hkv
    ng = B // GS
    gt = GS * Sq
    cw = rep * Dh
    bf = jnp.bfloat16
    any_spec = pl.BlockSpec(memory_space=pl.ANY)
    out = pl.pallas_call(
        functools.partial(_kernel, B=B, Sq=Sq),
        in_specs=[any_spec] * 5,
        out_specs=any_spec,
        out_shape=jax.ShapeDtypeStruct((B * Sq, D), x.dtype),
        scratch_shapes=[
            pltpu.VMEM((ng, gt, D), bf),
            pltpu.VMEM((Hkv, D, cw), bf),
            pltpu.VMEM((Hkv, D, cw), bf),
            pltpu.VMEM((GS, Hkv, rep * Sq, Dh), bf),
            pltpu.VMEM((GS, Hkv, rep * Sq, Dh), bf),
            pltpu.VMEM((Hkv, gt, cw), bf),
            pltpu.VMEM((Hkv, gt, cw), bf),
            pltpu.VMEM((gt // TT, D, TT), jnp.float32),
            pltpu.VMEM((gt // TT, D, TT), jnp.float32),
            pltpu.VMEM((ng, gt, D), bf),
            pltpu.VMEM((GS, Hkv, Sk, Dh), bf),
            pltpu.VMEM((GS, Hkv, Sk, Dh), bf),
            pltpu.SemaphoreType.DMA((ng + 1,)),
            pltpu.SemaphoreType.DMA((Hkv + 1,)),
            pltpu.SemaphoreType.DMA((Hkv,)),
            pltpu.SemaphoreType.DMA((2, GS // U)),
            pltpu.SemaphoreType.DMA((ng, gt // TT)),
        ],
        compiler_params=pltpu.CompilerParams(vmem_limit_bytes=120 * 1024 * 1024),
    )(x.reshape(B * Sq, D), k_cache, v_cache, wq, wo.T)
    return out.reshape(B, Sq, D)
```
